```python
import os as _os
_os.environ.setdefault("JAX_PLATFORMS", "cpu")
import jax
import jax.numpy as jnp

def _softmax(x, axis=-1):
    return jax.nn.softmax(x, axis=axis)
def _gelu(x):
    return jax.nn.gelu(x, approximate=True)
def _silu(x):
    return jax.nn.silu(x)
def _sigmoid(x):
    return jax.nn.sigmoid(x)
def _layernorm(x, axis=-1, eps=1e-5):
    m = jnp.mean(x, axis=axis, keepdims=True)
    v = jnp.var(x, axis=axis, keepdims=True)
    return (x - m) / jnp.sqrt(v + eps)
def _scatter_add(tgt, idx, src, axis=0):
    return tgt.at[idx].add(src)
def _segment_sum(src, seg, n):
    return jax.ops.segment_sum(src, seg, n)
class _Rng:
    def __init__(self, key):
        self._k = key
    def _next(self):
        self._k, sub = jax.random.split(self._k)
        return sub
    def normal(self, shape):
        return jax.random.normal(self._next(), shape, dtype=jnp.bfloat16)
    def randint(self, lo, hi, shape):
        return jax.random.randint(self._next(), shape, lo, hi, dtype=jnp.int32)
    def uniform(self, shape, lo=0.0, hi=1.0):
        return jax.random.uniform(self._next(), shape, jnp.bfloat16, lo, hi)
    def permutation(self, n):
        return jax.random.permutation(self._next(), n)


kernel_name = 'standalone__gqa_block_cached__sampling'

def setup_inputs():
    _rng = _Rng(jax.random.key(int.from_bytes(__import__("os").urandom(4), "little")))
    _w = (lambda a: (lambda t: t.astype(jnp.bfloat16) if jnp.issubdtype(t.dtype, jnp.floating) else t)(jnp.asarray(a)))
    B, Sq, D = 32, 16, 1024
    Hq, Hkv, Sk, Dh = 32, 4, 2048, 128
    assert Hq % Hkv == 0, (Hq, Hkv)
    return {
        "x": _w((lambda *s: _rng.normal(s) * 0.8)(B, Sq, D)),
        "k_cache": _w((lambda *s: _rng.normal(s) * 0.8)(B, Hkv, Sk, Dh)),
        "v_cache": _w((lambda *s: _rng.normal(s) * 0.05)(B, Hkv, Sk, Dh)),
        "wq": _w((lambda *s: _rng.normal(s) * 0.8)(D, Hq * Dh) * (D ** -0.5)),
        "wo": _w((lambda *s: _rng.normal(s) * 0.05)(Hq * Dh, D) * ((Hq * Dh) ** -0.5)),
    }

def reference(x, k_cache, v_cache, wq, wo):
    B, Sq, D = x.shape
    Hq, Dh = 32, 128
    Hkv = k_cache.shape[1]
    rep = Hq // Hkv
    q = (lambda x, *d: x.transpose(*d))((x @ wq).reshape(B, Sq, Hq, Dh), 0, 2, 1, 3)
    k = jnp.repeat(k_cache, rep, axis=1)
    v = jnp.repeat(v_cache, rep, axis=1)
    scores = jnp.einsum("bhqd,bhkd->bhqk", q, k) * (Dh ** -0.5)
    p = _softmax(scores, axis=-1)
    o = jnp.einsum("bhqk,bhkd->bhqd", p, v)
    return (lambda x, *d: x.transpose(*d))(o, 0, 2, 1, 3).reshape(B, Sq, Hq * Dh) @ wo
```

```python
import functools
import jax
import jax.numpy as jnp
import jax.experimental.pallas as pl
import jax.experimental.pallas.tpu as pltpu


def _kernel(x_ref, k_ref, v_ref, wq_ref, wo_ref, out_ref, q_scr, o_scr, *, Sq, Dh, rep, scale):
    b = pl.program_id(0)
    h = pl.program_id(1)
    nb = pl.num_programs(0)
    nh = pl.num_programs(1)
    G = rep * Dh

    @pl.when(jnp.logical_and(b == 0, h == 0))
    def _():
        NCH = q_scr.shape[1] // 512
        for c in range(NCH):
            q_scr[:, c * 512:(c + 1) * 512] = jnp.dot(
                x_ref[...], wq_ref[:, c * 512:(c + 1) * 512],
                preferred_element_type=jnp.float32).astype(q_scr.dtype)

    row0 = pl.multiple_of(b * Sq, Sq)
    col0 = pl.multiple_of(h * G, G)
    qb = q_scr[pl.ds(row0, Sq), pl.ds(col0, G)]
    q = jnp.concatenate([qb[:, i * Dh:(i + 1) * Dh] for i in range(rep)], axis=0)
    k = k_ref[0, 0]
    v = v_ref[0, 0]
    s = jax.lax.dot_general(q, k, (((1,), (1,)), ((), ())),
                            preferred_element_type=jnp.float32) * scale
    m = jnp.max(s, axis=1, keepdims=True)
    p = jnp.exp(s - m)
    l = jnp.sum(p, axis=1, keepdims=True)
    o = jnp.dot(p.astype(v.dtype), v, preferred_element_type=jnp.float32) / l
    o = o.astype(o_scr.dtype)
    ob = jnp.concatenate([o[i * Sq:(i + 1) * Sq, :] for i in range(rep)], axis=1)
    o_scr[pl.ds(row0, Sq), pl.ds(col0, G)] = ob

    @pl.when(jnp.logical_and(b == nb - 1, h == nh - 1))
    def _():
        NCH = out_ref.shape[1] // 256
        for c in range(NCH):
            out_ref[:, c * 256:(c + 1) * 256] = jnp.dot(
                o_scr[...], wo_ref[:, c * 256:(c + 1) * 256],
                preferred_element_type=jnp.float32).astype(out_ref.dtype)


@jax.jit
def pallas_standalone__gqa_block_cached__sampling_kernel(x, k_cache, v_cache, wq, wo):
    B, Sq, D = x.shape
    _, Hkv, Sk, Dh = k_cache.shape
    HD = wq.shape[1]
    Hq = HD // Dh
    rep = Hq // Hkv
    M = B * Sq
    x2 = x.reshape(M, D)
    kern = functools.partial(_kernel, Sq=Sq, Dh=Dh, rep=rep, scale=float(Dh) ** -0.5)
    out = pl.pallas_call(
        kern,
        grid=(B, Hkv),
        in_specs=[
            pl.BlockSpec((M, D), lambda b, h: (0, 0)),
            pl.BlockSpec((1, 1, Sk, Dh), lambda b, h: (b, h, 0, 0)),
            pl.BlockSpec((1, 1, Sk, Dh), lambda b, h: (b, h, 0, 0)),
            pl.BlockSpec((D, HD), lambda b, h: (0, 0)),
            pl.BlockSpec((HD, D), lambda b, h: (0, 0)),
        ],
        out_specs=pl.BlockSpec((M, D), lambda b, h: (0, 0)),
        out_shape=jax.ShapeDtypeStruct((M, D), x.dtype),
        scratch_shapes=[
            pltpu.VMEM((M, HD), jnp.bfloat16),
            pltpu.VMEM((M, HD), jnp.bfloat16),
        ],
        compiler_params=pltpu.CompilerParams(
            dimension_semantics=("arbitrary", "arbitrary"),
            vmem_limit_bytes=100 * 1024 * 1024,
        ),
    )(x2, k_cache, v_cache, wq, wo)
    return out.reshape(B, Sq, D)
```

```python
import functools
import math
import jax
import jax.numpy as jnp
import jax.experimental.pallas as pl
import jax.experimental.pallas.tpu as pltpu

BB = 4


def _kernel(x_ref, k_ref, v_ref, wq0_ref, wqs_ref, wos_ref, wol_ref, out_ref,
            q_scr, o_scr, qacc, oacc, *, Sq, Dh, rep, scale, KC, NC, BB):
    h = pl.program_id(0)
    bi = pl.program_id(1)
    nh = pl.num_programs(0)
    nb = pl.num_programs(1)
    G = rep * Dh
    nkk = G // KC
    HD = o_scr.shape[1]
    R = BB * Sq

    def qproj_rows(r):
        rr = pl.multiple_of(r * R, R)
        q_scr[pl.ds(rr, R), 0:G] = jnp.dot(
            x_ref[pl.ds(rr, R), :], wq0_ref[...],
            preferred_element_type=jnp.float32).astype(q_scr.dtype)

    def oproj_rows(r, valid):
        rr = pl.multiple_of(r * R, R)
        part = jnp.dot(o_scr[pl.ds(rr, R), HD - G:HD], wol_ref[...],
                       preferred_element_type=jnp.float32)
        oacc[pl.ds(rr, R), :] += jnp.where(valid, part, 0.0)

    @pl.when(jnp.logical_and(bi == 0, h == 0))
    def _():
        qproj_rows(0)
        oacc[...] = jnp.zeros(oacc.shape, oacc.dtype)
        qacc[...] = jnp.zeros(qacc.shape, qacc.dtype)

    col0 = pl.multiple_of(h * G, G)
    c2 = scale * math.log2(math.e)
    for j in range(BB):
        row0 = pl.multiple_of((bi * BB + j) * Sq, Sq)
        qb = q_scr[pl.ds(row0, Sq), pl.ds(col0, G)]
        q = jnp.concatenate([qb[:, i * Dh:(i + 1) * Dh] for i in range(rep)], axis=0)
        k = k_ref[j, 0]
        v = v_ref[j, 0]
        s = jax.lax.dot_general(q, k, (((1,), (1,)), ((), ())),
                                preferred_element_type=jnp.float32)
        m = jnp.max(s, axis=1, keepdims=True)
        p = jnp.exp2((s - m) * c2)
        l = jnp.sum(p, axis=1, keepdims=True)
        o = jnp.dot(p.astype(v.dtype), v, preferred_element_type=jnp.float32) / l
        o = o.astype(o_scr.dtype)
        ob = jnp.concatenate([o[i * Sq:(i + 1) * Sq, :] for i in range(rep)], axis=1)
        o_scr[pl.ds(row0, Sq), pl.ds(col0, G)] = ob

    kk = bi % nkk
    c = bi // nkk

    xk = x_ref[:, pl.ds(pl.multiple_of(kk * KC, KC), KC)]
    part = jnp.dot(xk, wqs_ref[...], preferred_element_type=jnp.float32)
    if nkk > 1:
        acc = jnp.where(kk > 0, qacc[...], 0.0) + part
        qacc[...] = acc
    else:
        acc = part
    valid = jnp.logical_and(h < nh - 1, kk == nkk - 1)
    qcol = jnp.where(valid, (h + 1) * G + c * NC, HD)
    q_scr[:, pl.ds(pl.multiple_of(qcol, NC), NC)] = acc.astype(q_scr.dtype)

    gcol = jnp.maximum(h - 1, 0) * G
    ok = o_scr[:, pl.ds(pl.multiple_of(gcol + kk * KC, KC), KC)]
    part2 = jnp.dot(ok, wos_ref[...], preferred_element_type=jnp.float32)
    cc = pl.multiple_of(c * NC, NC)
    oacc[:, pl.ds(cc, NC)] += jnp.where(h > 0, part2, 0.0)

    @pl.when(h == 0)
    def _():
        qproj_rows(jnp.minimum(bi + 1, nb - 1))

    @pl.when(h == nh - 1)
    def _():
        oproj_rows(jnp.maximum(bi - 1, 0), bi > 0)

    @pl.when(jnp.logical_and(bi == nb - 1, h == nh - 1))
    def _():
        oproj_rows(nb - 1, True)
        out_ref[...] = oacc[...].astype(out_ref.dtype)


@jax.jit
def pallas_standalone__gqa_block_cached__sampling_kernel(x, k_cache, v_cache, wq, wo):
    B, Sq, D = x.shape
    _, Hkv, Sk, Dh = k_cache.shape
    HD = wq.shape[1]
    Hq = HD // Dh
    rep = Hq // Hkv
    M = B * Sq
    G = rep * Dh
    NC = 128
    ncg = G // NC
    nsteps = B // BB
    nkk = nsteps // ncg
    KC = G // nkk
    assert nsteps == nkk * ncg and nkk >= 1
    x2 = x.reshape(M, D)
    kern = functools.partial(_kernel, Sq=Sq, Dh=Dh, rep=rep, scale=float(Dh) ** -0.5, KC=KC, NC=NC, BB=BB)

    def wqs_map(h, b):
        last = h >= Hkv - 1
        return (jnp.where(last, nkk - 1, b % nkk),
                jnp.where(last, Hkv * ncg - 1, (h + 1) * ncg + b // nkk))

    def wos_map(h, b):
        first = h == 0
        return (jnp.where(first, 0, (h - 1) * nkk + b % nkk),
                jnp.where(first, 0, b // nkk))

    out = pl.pallas_call(
        kern,
        grid=(Hkv, nsteps),
        in_specs=[
            pl.BlockSpec((M, D), lambda h, b: (0, 0)),
            pl.BlockSpec((BB, 1, Sk, Dh), lambda h, b: (b, h, 0, 0)),
            pl.BlockSpec((BB, 1, Sk, Dh), lambda h, b: (b, h, 0, 0)),
            pl.BlockSpec((D, G), lambda h, b: (0, 0)),
            pl.BlockSpec((KC, NC), wqs_map),
            pl.BlockSpec((KC, NC), wos_map),
            pl.BlockSpec((G, D), lambda h, b: (Hkv - 1, 0)),
        ],
        out_specs=pl.BlockSpec((M, D), lambda h, b: (0, 0)),
        out_shape=jax.ShapeDtypeStruct((M, D), x.dtype),
        scratch_shapes=[
            pltpu.VMEM((M, HD + NC), jnp.bfloat16),
            pltpu.VMEM((M, HD), jnp.bfloat16),
            pltpu.VMEM((M, NC), jnp.float32),
            pltpu.VMEM((M, D), jnp.float32),
        ],
        compiler_params=pltpu.CompilerParams(
            dimension_semantics=("arbitrary", "arbitrary"),
            vmem_limit_bytes=100 * 1024 * 1024,
        ),
    )(x2, k_cache, v_cache, wq, wq, wo, wo)
    return out.reshape(B, Sq, D)
```

```python
import functools
import math

import jax
import jax.numpy as jnp
import jax.experimental.pallas as pl
import jax.experimental.pallas.tpu as pltpu

_BB = 4


def _kernel(x_ref, k_ref, v_ref, wq0_ref, wqs_ref, wos_ref, wol_ref, out_ref,
            q_scr, o_scr, oacc, *, Sq, Dh, rep, scale, NC, BB):
    h = pl.program_id(0)
    bi = pl.program_id(1)
    nh = pl.num_programs(0)
    nb = pl.num_programs(1)
    G = rep * Dh
    HD = o_scr.shape[1]
    R = BB * Sq

    def qproj_rows(r):
        rr = pl.multiple_of(r * R, R)
        q_scr[pl.ds(rr, R), 0:G] = jnp.dot(
            x_ref[pl.ds(rr, R), :], wq0_ref[...],
            preferred_element_type=jnp.float32).astype(q_scr.dtype)

    def oproj_rows(r, valid):
        rr = pl.multiple_of(r * R, R)
        part = jnp.dot(o_scr[pl.ds(rr, R), HD - G:HD], wol_ref[...],
                       preferred_element_type=jnp.float32)
        oacc[pl.ds(rr, R), :] += jnp.where(valid, part, 0.0)

    @pl.when(jnp.logical_and(bi == 0, h == 0))
    def _():
        qproj_rows(0)
        oacc[...] = jnp.zeros(oacc.shape, oacc.dtype)

    col0 = pl.multiple_of(h * G, G)
    c2 = scale * math.log2(math.e)
    for j in range(BB):
        row0 = pl.multiple_of((bi * BB + j) * Sq, Sq)
        qb = q_scr[pl.ds(row0, Sq), pl.ds(col0, G)]
        q = jnp.concatenate([qb[:, i * Dh:(i + 1) * Dh] for i in range(rep)], axis=0)
        k = k_ref[j, 0]
        v = v_ref[j, 0]
        s = jax.lax.dot_general(q, k, (((1,), (1,)), ((), ())),
                                preferred_element_type=jnp.float32)
        m = jnp.max(s, axis=1, keepdims=True)
        p = jnp.exp2((s - m) * c2)
        l = jnp.sum(p, axis=1, keepdims=True)
        o = jnp.dot(p.astype(v.dtype), v, preferred_element_type=jnp.float32) / l
        o = o.astype(o_scr.dtype)
        ob = jnp.concatenate([o[i * Sq:(i + 1) * Sq, :] for i in range(rep)], axis=1)
        o_scr[pl.ds(row0, Sq), pl.ds(col0, G)] = ob

    gcol = pl.multiple_of(jnp.maximum(h - 1, 0) * G, G)
    part2 = jnp.dot(o_scr[:, pl.ds(gcol, G)], wos_ref[...],
                    preferred_element_type=jnp.float32)
    cc = pl.multiple_of(bi * NC, NC)
    oacc[:, pl.ds(cc, NC)] += jnp.where(h > 0, part2, 0.0)

    @pl.when(h < nh - 1)
    def _():
        qcol = pl.multiple_of((h + 1) * G + bi * NC, NC)
        q_scr[:, pl.ds(qcol, NC)] = jnp.dot(
            x_ref[...], wqs_ref[...],
            preferred_element_type=jnp.float32).astype(q_scr.dtype)

    @pl.when(h == 0)
    def _():
        qproj_rows(jnp.minimum(bi + 1, nb - 1))

    @pl.when(h == nh - 1)
    def _():
        oproj_rows(jnp.maximum(bi - 1, 0), bi > 0)

    @pl.when(jnp.logical_and(bi == nb - 1, h == nh - 1))
    def _():
        oproj_rows(nb - 1, True)
        out_ref[...] = oacc[...].astype(out_ref.dtype)


@jax.jit
def pallas_standalone__gqa_block_cached__sampling_kernel(
    x: jax.Array,
    k_cache: jax.Array,
    v_cache: jax.Array,
    wq: jax.Array,
    wo: jax.Array,
):
    B, Sq, D = x.shape
    _, Hkv, Sk, Dh = k_cache.shape
    HD = wq.shape[1]
    Hq = HD // Dh
    rep = Hq // Hkv
    M = B * Sq
    G = rep * Dh
    BB = _BB
    nsteps = B // BB
    NC = G // nsteps
    assert B % BB == 0 and G % nsteps == 0 and D == G and NC % 128 == 0
    x2 = x.reshape(M, D)
    kern = functools.partial(_kernel, Sq=Sq, Dh=Dh, rep=rep, scale=float(Dh) ** -0.5,
                             NC=NC, BB=BB)

    def wqs_map(h, b):
        return (0, jnp.where(h >= Hkv - 1, Hkv * nsteps - 1, (h + 1) * nsteps + b))

    def wos_map(h, b):
        return (jnp.maximum(h - 1, 0), jnp.where(h == 0, 0, b))

    out = pl.pallas_call(
        kern,
        grid=(Hkv, nsteps),
        in_specs=[
            pl.BlockSpec((M, D), lambda h, b: (0, 0)),
            pl.BlockSpec((BB, 1, Sk, Dh), lambda h, b: (b, h, 0, 0)),
            pl.BlockSpec((BB, 1, Sk, Dh), lambda h, b: (b, h, 0, 0)),
            pl.BlockSpec((D, G), lambda h, b: (0, 0)),
            pl.BlockSpec((D, NC), wqs_map),
            pl.BlockSpec((G, NC), wos_map),
            pl.BlockSpec((G, D), lambda h, b: (Hkv - 1, 0)),
        ],
        out_specs=pl.BlockSpec((M, D), lambda h, b: (0, 0)),
        out_shape=jax.ShapeDtypeStruct((M, D), x.dtype),
        scratch_shapes=[
            pltpu.VMEM((M, HD), jnp.bfloat16),
            pltpu.VMEM((M, HD), jnp.bfloat16),
            pltpu.VMEM((M, D), jnp.float32),
        ],
        compiler_params=pltpu.CompilerParams(
            dimension_semantics=("arbitrary", "arbitrary"),
            vmem_limit_bytes=100 * 1024 * 1024,
        ),
    )(x2, k_cache, v_cache, wq, wq, wo, wo)
    return out.reshape(B, Sq, D)
```
